```python
import os as _os
_os.environ.setdefault("JAX_PLATFORMS", "cpu")
import jax
import jax.numpy as jnp

def _softmax(x, axis=-1):
    return jax.nn.softmax(x, axis=axis)
def _gelu(x):
    return jax.nn.gelu(x, approximate=True)
def _silu(x):
    return jax.nn.silu(x)
def _sigmoid(x):
    return jax.nn.sigmoid(x)
def _layernorm(x, axis=-1, eps=1e-5):
    m = jnp.mean(x, axis=axis, keepdims=True)
    v = jnp.var(x, axis=axis, keepdims=True)
    return (x - m) / jnp.sqrt(v + eps)
def _scatter_add(tgt, idx, src, axis=0):
    return tgt.at[idx].add(src)
def _segment_sum(src, seg, n):
    return jax.ops.segment_sum(src, seg, n)
class _Rng:
    def __init__(self, key):
        self._k = key
    def _next(self):
        self._k, sub = jax.random.split(self._k)
        return sub
    def normal(self, shape):
        return jax.random.normal(self._next(), shape, dtype=jnp.bfloat16)
    def randint(self, lo, hi, shape):
        return jax.random.randint(self._next(), shape, lo, hi, dtype=jnp.int32)
    def uniform(self, shape, lo=0.0, hi=1.0):
        return jax.random.uniform(self._next(), shape, jnp.bfloat16, lo, hi)
    def permutation(self, n):
        return jax.random.permutation(self._next(), n)


kernel_name = 'standalone__dcn_v2_cross__recsys'

def setup_inputs():
    _rng = _Rng(jax.random.key(int.from_bytes(__import__("os").urandom(4), "little")))
    _w = (lambda a: (lambda t: t.astype(jnp.bfloat16) if jnp.issubdtype(t.dtype, jnp.floating) else t)(jnp.asarray(a)))
    B, F, D, L = 4096, 26, 128, 6
    Din = min(F * D, 1024)
    return {
        "x0": _w((lambda *s: _rng.normal(s) * 0.05)(B, Din)),
        "ws": _w((lambda *s: _rng.normal(s) * 0.05)(L, Din, Din)),
        "bs": _w((lambda *s: _rng.normal(s) * 0.05)(L, Din)),
    }

def reference(x0, ws, bs):
    x = x0
    for l in range(ws.shape[0]):
        x = x0 * (x @ ws[l] + bs[l]) + x
    return x
```

```python
import jax
import jax.numpy as jnp
import jax.experimental.pallas as pl
import jax.experimental.pallas.tpu as pltpu

f32 = jnp.float32

BM = 512
K_CHUNKS = (128, 256, 256, 384)
OC = 256


def _kernel(x0_hbm, w_hbm, b_hbm, o_hbm,
            w_v, b_v, bias, x_v, o_v, xf, xb1, xb2,
            wsem, bsem, xsem, osem, csem):
    L, D, _ = w_hbm.shape
    B = x0_hbm.shape[0]
    dt = x_v.dtype
    nk = len(K_CHUNKS)
    kslice = [pl.ds(sum(K_CHUNKS[:k]), K_CHUNKS[k]) for k in range(nk)]
    first = pl.ds(0, BM)
    rest = pl.ds(BM, B - BM)

    def wcopy(l):
        return pltpu.make_async_copy(w_hbm.at[l], w_v.at[l], wsem.at[l])

    def xk(k):
        return pltpu.make_async_copy(
            x0_hbm.at[first, kslice[k]], x_v.at[first, kslice[k]], csem.at[0, k])

    def wk(k):
        return pltpu.make_async_copy(
            w_hbm.at[0, kslice[k]], w_v.at[0, kslice[k]], csem.at[1, k])

    xrest = pltpu.make_async_copy(x0_hbm.at[rest], x_v.at[rest], xsem)
    bcopy = pltpu.make_async_copy(b_hbm, b_v, bsem)

    for k in range(nk):
        xk(k).start()
        wk(k).start()
    bcopy.start()

    for k in range(nk):
        xk(k).wait()
        wk(k).wait()
        if k == 0:
            wcopy(1).start()
        if k == nk - 1:
            bcopy.wait()
        p = jnp.dot(x_v[first, kslice[k]], w_v[0, kslice[k], :],
                    preferred_element_type=f32)
        y = p if k == 0 else xf[...] + p
        if k < nk - 1:
            xf[...] = y
    for l in range(L):
        bias[l] = b_v[l:l + 1, :].astype(f32)
    x0 = x_v[first].astype(f32)
    x = x0 * (y + bias[0]) + x0
    xf[...] = x
    xb1[...] = x.astype(dt)

    for l in range(2, L):
        wcopy(l).start()
    xrest.start()

    def layer(l, _):
        wcopy(l).wait()
        y = jnp.dot(xb1[...], w_v[l], preferred_element_type=f32)
        x = x_v[first].astype(f32) * (y + bias[l]) + xf[...]
        xf[...] = x
        xb1[...] = x.astype(dt)

    jax.lax.fori_loop(1, L, layer, None)
    pltpu.make_async_copy(xb1, o_hbm.at[first], osem).start()
    xrest.wait()

    def block(i, _):
        orows = pl.ds(pl.multiple_of(i * BM, BM), BM)
        rows = pl.ds(pl.multiple_of((i + 1) * BM, BM), BM)
        for l in range(L):
            xb = x_v[rows] if l == 0 else xb2[l % 2]
            for j in range(D // OC):
                c = slice(j * OC, (j + 1) * OC)
                y = jnp.dot(xb, w_v[l, :, c], preferred_element_type=f32)
                x0 = x_v[rows, c].astype(f32)
                x = x0 * (y + bias[l, :, c]) + (x0 if l == 0 else xf[:, c])
                if l < L - 1:
                    xf[:, c] = x
                    xb2[(l + 1) % 2, :, c] = x.astype(dt)
                else:
                    o_v[orows, c] = x.astype(dt)
                    pltpu.make_async_copy(
                        o_v.at[orows, c], o_hbm.at[rows, c], osem).start()

    jax.lax.fori_loop(0, B // BM - 1, block, None)
    pltpu.make_async_copy(x_v, o_hbm, osem).wait()


@jax.jit
def pallas_standalone__dcn_v2_cross__recsys_kernel(
    x0: jax.Array,
    ws: jax.Array,
    bs: jax.Array,
):
    B, D = x0.shape
    L = ws.shape[0]
    assert B % BM == 0 and B > BM and sum(K_CHUNKS) == D and D % OC == 0 and L >= 2
    return pl.pallas_call(
        _kernel,
        in_specs=[pl.BlockSpec(memory_space=pl.ANY)] * 3,
        out_specs=pl.BlockSpec(memory_space=pl.ANY),
        out_shape=jax.ShapeDtypeStruct((B, D), x0.dtype),
        scratch_shapes=[
            pltpu.VMEM((L, D, D), ws.dtype),
            pltpu.VMEM((L, D), bs.dtype),
            pltpu.VMEM((L, 1, D), f32),
            pltpu.VMEM((B, D), x0.dtype),
            pltpu.VMEM((B - BM, D), x0.dtype),
            pltpu.VMEM((BM, D), f32),
            pltpu.VMEM((BM, D), x0.dtype),
            pltpu.VMEM((2, BM, D), x0.dtype),
            pltpu.SemaphoreType.DMA((L,)),
            pltpu.SemaphoreType.DMA(()),
            pltpu.SemaphoreType.DMA(()),
            pltpu.SemaphoreType.DMA(()),
            pltpu.SemaphoreType.DMA((2, len(K_CHUNKS))),
        ],
        compiler_params=pltpu.CompilerParams(vmem_limit_bytes=100 * 1024 * 1024),
    )(x0, ws, bs)
```
